```python
import os as _os
_os.environ.setdefault('JAX_PLATFORMS', 'cpu')
import jax
import jax.numpy as jnp

def _softmax(x, axis=-1):
    return jax.nn.softmax(x, axis=axis)

def _gelu(x):
    return jax.nn.gelu(x, approximate=True)

def _silu(x):
    return jax.nn.silu(x)

def _sigmoid(x):
    return jax.nn.sigmoid(x)

def _layernorm(x, axis=-1, eps=1e-05):
    m = jnp.mean(x, axis=axis, keepdims=True)
    v = jnp.var(x, axis=axis, keepdims=True)
    return (x - m) / jnp.sqrt(v + eps)

def _scatter_add(tgt, idx, src, axis=0):
    return tgt.at[idx].add(src)

def _segment_sum(src, seg, n):
    return jax.ops.segment_sum(src, seg, n)

class _Rng:

    def __init__(self, key):
        self._k = key

    def _next(self):
        self._k, sub = jax.random.split(self._k)
        return sub

    def normal(self, shape):
        return jax.random.normal(self._next(), shape, dtype=jnp.bfloat16)

    def randint(self, lo, hi, shape):
        return jax.random.randint(self._next(), shape, lo, hi, dtype=jnp.int32)

    def uniform(self, shape, lo=0.0, hi=1.0):
        return jax.random.uniform(self._next(), shape, jnp.bfloat16, lo, hi)

    def permutation(self, n):
        return jax.random.permutation(self._next(), n)
kernel_name = 'adaLN_cond__mha_block__dense_activation_squared_relu__prompt'

def setup_inputs():
    _rng = _Rng(jax.random.key(int.from_bytes(__import__("os").urandom(4), "little")))
    _w = lambda a: (lambda t: t.astype(jnp.bfloat16) if jnp.issubdtype(t.dtype, jnp.floating) else t)(jnp.asarray(a))

    def _A_setup():
        B, S, D, H = (1, 2048, 512, 32)
        return {'x': _w((lambda *s: _rng.normal(s) * 0.05)(B, S, D)), 'wqkv': _w((lambda *s: _rng.normal(s) * 0.1)(D, 3 * D)), 'wo': _w((lambda *s: _rng.normal(s) * 0.05)(D, D))}
    _A_in = _A_setup()

    def _B_setup():
        B, S, D, F = (1, 2048, 512, 1792)
        return {'x': _w((lambda *s: _rng.normal(s) * 0.05)(B, S, D)), 'w1': _w((lambda *s: _rng.normal(s) * 0.05)(D, F)), 'b1': _w((lambda *s: _rng.normal(s) * 0.05)(F)), 'w2': _w((lambda *s: _rng.normal(s) * 0.05)(F, D)), 'b2': _w((lambda *s: _rng.normal(s) * 0.05)(D))}
    _B_in = _B_setup()
    return {'A_x': _A_in['x'], 'A_wqkv': _A_in['wqkv'], 'A_wo': _A_in['wo'], 'B_x': _B_in['x'], 'B_w1': _B_in['w1'], 'B_b1': _B_in['b1'], 'B_w2': _B_in['w2'], 'B_b2': _B_in['b2'], 'c': _w((lambda *s: _rng.normal(s) * 0.05)(1, 512) * 8.0), 'w_mod': _w((lambda *s: _rng.normal(s) * 0.05)(512, 6 * 512) * 512 ** (-0.5) * 8.0)}

def reference(A_x, A_wqkv, A_wo, B_x, B_w1, B_b1, B_w2, B_b2, c, w_mod):

    def _A_ref(x, wqkv, wo):
        B, S, D = x.shape
        H = 32
        Dh = D // H
        qkv = (lambda x, *d: x.transpose(*d))((x @ wqkv).reshape(B, S, 3, H, Dh), 2, 0, 3, 1, 4)
        q, k, v = (qkv[0], qkv[1], qkv[2])
        scores = jnp.einsum('bhqd,bhkd->bhqk', q, k) * Dh ** (-0.5)
        p = _softmax(scores, axis=-1)
        o = jnp.einsum('bhqk,bhkd->bhqd', p, v)
        return (lambda x, *d: x.transpose(*d))(o, 0, 2, 1, 3).reshape(B, S, D) @ wo

    def _B_ref(x, w1, b1, w2, b2):
        h = jnp.einsum('bsd,df->bsf', x, w1) + b1
        zero = jnp.zeros_like(h)
        r = jnp.where(h > zero, h, zero)
        h = r * r
        out = jnp.einsum('bsf,fd->bsd', h, w2) + b2
        return out
    x = A_x
    mod = (_silu(c) @ w_mod).reshape(c.shape[0], 6, 1, -1)
    sa, ca, ga, sb, cb, gb = (mod[:, 0].copy(), mod[:, 1].copy(), mod[:, 2].copy(), mod[:, 3].copy(), mod[:, 4].copy(), mod[:, 5].copy())
    h = _layernorm(x, axis=-1) * (1 + ca) + sa
    x = x + ga * _A_ref(h, A_wqkv, A_wo)
    h = _layernorm(x, axis=-1) * (1 + cb) + sb
    x = x + gb * _B_ref(h, B_w1, B_b1, B_w2, B_b2)
    return x
```

```python
import functools
import math

import jax
import jax.numpy as jnp
import jax.experimental.pallas as pl
import jax.experimental.pallas.tpu as pltpu

f32 = jnp.float32
bf16 = jnp.bfloat16

_H = 32
_EPS = 1e-5
_TQ = 512
_CK = 128
_RC = 256
_FC = 256


def _layernorm(xf):
    mu = jnp.mean(xf, axis=-1, keepdims=True)
    xc = xf - mu
    var = jnp.mean(xc * xc, axis=-1, keepdims=True)
    return xc * jax.lax.rsqrt(var + _EPS)


def _kernel(x_ref, wk_ref, wqvt_ref, wo_ref, w1_ref, b1_ref, w2_ref, b2_ref, c_ref, wmod_ref,
            o_ref,
            mod_scr, k_scr, qt_scr, vt_scr, qm_scr, sA, sB, ot_scr, *, S, D, F):
    t = pl.program_id(0)
    H = _H
    Dh = D // H
    G = 128 // Dh
    NG = D // 128
    TQ, CK = _TQ, _CK
    NC = S // CK
    qscale = (Dh ** -0.5) * math.log2(math.e)

    @pl.when(t == 0)
    def _prologue():
        cf = c_ref[...].astype(f32)
        sc = cf * jax.nn.sigmoid(cf)
        sc8 = jnp.broadcast_to(sc, (16, D)).astype(bf16)
        mod = jnp.dot(sc8, wmod_ref[...], preferred_element_type=f32)
        mod_scr[...] = mod[0:8, :]
        qm_scr[...] = jnp.zeros(qm_scr.shape, qm_scr.dtype)
        vt_scr[:, Dh:2 * Dh, :] = jnp.ones((H, Dh, S), bf16)

        sa = mod[0:1, 0:D]
        ca1 = 1.0 + mod[0:1, D:2 * D]

        def rows(r, carry):
            r0 = pl.multiple_of(r * _RC, _RC)
            xf = x_ref[pl.ds(r0, _RC), :].astype(f32)
            h = (_layernorm(xf) * ca1 + sa).astype(bf16)
            k = jnp.dot(h, wk_ref[...], preferred_element_type=f32).astype(bf16)
            for g in range(NG):
                k_scr[g, pl.ds(r0, _RC), :] = k[:, 128 * g:128 * (g + 1)]
            qv = jax.lax.dot_general(wqvt_ref[...], h, (((1,), (1,)), ((), ())),
                                     preferred_element_type=f32)
            qt_scr[:, pl.ds(r0, _RC)] = (qv[0:D, :] * qscale).astype(bf16)
            vt_scr[:, 0:Dh, pl.ds(r0, _RC)] = qv[D:2 * D, :].astype(bf16).reshape(H, Dh, _RC)
            return carry

        jax.lax.fori_loop(0, S // _RC, rows, 0)

    q0 = pl.multiple_of(t * TQ, TQ)
    for h in range(H):
        j = h % G
        qm_scr[h, Dh * j:Dh * (j + 1), :] = qt_scr[Dh * h:Dh * (h + 1), pl.ds(q0, TQ)]

    def qk_chunk(u, buf, c, m):
        kc = k_scr[u // G, c * CK:(c + 1) * CK, :]
        s = jnp.dot(kc, qm_scr[u], preferred_element_type=f32)
        buf[c * CK:(c + 1) * CK, :] = s
        return jnp.maximum(m, s.reshape(CK // 8, 8, TQ).max(axis=0))

    def pv_chunk(u, buf, c, mb, o):
        p = jnp.exp2(buf[c * CK:(c + 1) * CK, :] - mb).astype(bf16)
        vt = vt_scr[u, :, c * CK:(c + 1) * CK]
        return o + jnp.dot(vt, p, preferred_element_type=f32)

    neg = jnp.full((8, TQ), -jnp.inf, f32)

    def stage(u, cur, nxt, m, do_next=True):
        mb = m.max(axis=0, keepdims=True)
        o = jnp.zeros((2 * Dh, TQ), f32)
        mn = neg
        for c in range(NC):
            if do_next:
                mn = qk_chunk(u + 1, nxt, c, mn)
            o = pv_chunk(u, cur, c, mb, o)
        r = o[0:Dh, :] / o[Dh:Dh + 1, :]
        ot_scr[pl.ds(pl.multiple_of(u * Dh, Dh), Dh), :] = r.astype(ot_scr.dtype)
        return mn

    m = neg
    for c in range(NC):
        m = qk_chunk(0, sA, c, m)

    def body(i, m):
        m = stage(2 * i, sA, sB, m)
        return stage(2 * i + 1, sB, sA, m)

    m = jax.lax.fori_loop(0, H // 2 - 1, body, m)
    m = stage(H - 2, sA, sB, m)
    stage(H - 1, sB, sA, m, do_next=False)

    ga = mod_scr[0:1, 2 * D:3 * D]
    sb = mod_scr[0:1, 3 * D:4 * D]
    cb1 = 1.0 + mod_scr[0:1, 4 * D:5 * D]
    gb = mod_scr[0:1, 5 * D:6 * D]

    o_nat = ot_scr[...].T.astype(bf16)
    attn = jnp.dot(o_nat, wo_ref[...], preferred_element_type=f32)
    x1 = x_ref[pl.ds(q0, TQ), :].astype(f32) + ga * attn
    h2 = (_layernorm(x1) * cb1 + sb).astype(bf16)
    acc = jnp.zeros((TQ, D), f32)
    for fc in range(F // _FC):
        u = jnp.dot(h2, w1_ref[:, fc * _FC:(fc + 1) * _FC], preferred_element_type=f32)
        u = u + b1_ref[:, fc * _FC:(fc + 1) * _FC].astype(f32)
        r = jnp.maximum(u, 0.0)
        acc = acc + jnp.dot((r * r).astype(bf16), w2_ref[fc * _FC:(fc + 1) * _FC, :],
                            preferred_element_type=f32)
    out = x1 + gb * (acc + b2_ref[...].astype(f32))
    o_ref[...] = out.astype(o_ref.dtype)


@jax.jit
def pallas_adaLN_cond__mha_block__dense_activation_squared_relu__prompt_kernel(
    A_x: jax.Array,
    A_wqkv: jax.Array,
    A_wo: jax.Array,
    B_x: jax.Array,
    B_w1: jax.Array,
    B_b1: jax.Array,
    B_w2: jax.Array,
    B_b2: jax.Array,
    c: jax.Array,
    w_mod: jax.Array,
):
    B, S, D = A_x.shape
    F = B_w1.shape[1]
    H = _H
    Dh = D // H
    x = A_x.reshape(S, D)
    wk = A_wqkv[:, D:2 * D]
    wqvt = jnp.concatenate([A_wqkv[:, 0:D], A_wqkv[:, 2 * D:3 * D]], axis=1).T
    b1 = B_b1.reshape(1, F)
    b2 = B_b2.reshape(1, D)

    def full(shape):
        return pl.BlockSpec(shape, lambda t: (0,) * len(shape))

    out = pl.pallas_call(
        functools.partial(_kernel, S=S, D=D, F=F),
        grid=(S // _TQ,),
        in_specs=[full((S, D)), full((D, D)), full((2 * D, D)), full((D, D)),
                  full((D, F)), full((1, F)), full((F, D)), full((1, D)),
                  full((1, D)), full((D, 6 * D))],
        out_specs=pl.BlockSpec((_TQ, D), lambda t: (t, 0)),
        out_shape=jax.ShapeDtypeStruct((S, D), A_x.dtype),
        scratch_shapes=[
            pltpu.VMEM((8, 6 * D), f32),
            pltpu.VMEM((D // 128, S, 128), bf16),
            pltpu.VMEM((D, S), bf16),
            pltpu.VMEM((H, 2 * Dh, S), bf16),
            pltpu.VMEM((H, 128, _TQ), bf16),
            pltpu.VMEM((S, _TQ), f32),
            pltpu.VMEM((S, _TQ), f32),
            pltpu.VMEM((D, _TQ), f32),
        ],
        compiler_params=pltpu.CompilerParams(
            dimension_semantics=("arbitrary",),
            vmem_limit_bytes=100 * 1024 * 1024,
        ),
    )(x, wk, wqvt, A_wo, B_w1, b1, B_w2, b2, c, w_mod)
    return out.reshape(B, S, D)
```

```python
import functools
import math

import jax
import jax.numpy as jnp
import jax.experimental.pallas as pl
import jax.experimental.pallas.tpu as pltpu

f32 = jnp.float32
bf16 = jnp.bfloat16

_H = 32
_EPS = 1e-5
_TQ = 512
_CK = 128
_RC = 256
_FC = 256
_TIE = 4
_U = 4


def _layernorm(xf):
    mu = jnp.mean(xf, axis=-1, keepdims=True)
    xc = xf - mu
    var = jnp.mean(xc * xc, axis=-1, keepdims=True)
    return xc * jax.lax.rsqrt(var + _EPS)


def _kernel(x_hbm, wqkv_hbm, wo_hbm, w1_hbm, b1_ref, w2_hbm, b2_ref, c_ref, wmod_hbm,
            o_ref,
            x_ref, wqkv_ref, wo_ref, w1_ref, w2_ref, wmod_ref, sems, xsems,
            wqvt_ref, mod_scr, k_scr, qt_scr, vt_scr, qm_scr, sA, sB, ot_scr, *, S, D, F):
    t = pl.program_id(0)
    H = _H
    Dh = D // H
    G = 128 // Dh
    NG = D // 128
    TQ, CK = _TQ, _CK
    NC = S // CK
    qscale = (Dh ** -0.5) * math.log2(math.e)

    NR = S // _RC

    def late_copies():
        return [pltpu.make_async_copy(src, dst, sems.at[i]) for i, (src, dst) in enumerate(
            [(wmod_hbm.at[:, 2 * D:6 * D], wmod_ref.at[:, 2 * D:6 * D]),
             (wo_hbm, wo_ref), (w1_hbm, w1_ref), (w2_hbm, w2_ref)])]

    def x_copy(r):
        return pltpu.make_async_copy(x_hbm.at[0, pl.ds(r * _RC, _RC), :],
                                     x_ref.at[pl.ds(r * _RC, _RC), :], xsems.at[r])

    def silu_c():
        cf = c_ref[...].astype(f32)
        return jnp.broadcast_to(cf * jax.nn.sigmoid(cf), (16, D)).astype(bf16)

    @pl.when(t == 0)
    def _prologue():
        cp_mod = pltpu.make_async_copy(wmod_hbm.at[:, 0:2 * D], wmod_ref.at[:, 0:2 * D], sems.at[4])
        cp_qkv = pltpu.make_async_copy(wqkv_hbm, wqkv_ref, sems.at[5])
        cp_qkv.start()
        cp_mod.start()
        for r in range(NR):
            x_copy(r).start()
        qm_scr[...] = jnp.zeros(qm_scr.shape, qm_scr.dtype)
        cp_qkv.wait()
        wqvt_ref[0:D, :] = wqkv_ref[:, 0:D].T
        wqvt_ref[D:2 * D, :] = wqkv_ref[:, 2 * D:3 * D].T
        cp_mod.wait()
        mod = jnp.dot(silu_c(), wmod_ref[:, 0:2 * D], preferred_element_type=f32)
        for cp in late_copies():
            cp.start()

        sa = mod[0:1, 0:D]
        ca1 = 1.0 + mod[0:1, D:2 * D]

        def rows(r, carry):
            r0 = pl.multiple_of(r * _RC, _RC)
            x_copy(r).wait()
            xf = x_ref[pl.ds(r0, _RC), :].astype(f32)
            h = (_layernorm(xf) * ca1 + sa).astype(bf16)
            k = jnp.dot(h, wqkv_ref[:, D:2 * D], preferred_element_type=f32).astype(bf16)
            for g in range(NG):
                k_scr[g, pl.ds(r0, _RC), :] = k[:, 128 * g:128 * (g + 1)]
            qv = jax.lax.dot_general(wqvt_ref[...], h, (((1,), (1,)), ((), ())),
                                     preferred_element_type=f32)
            qt_scr[:, pl.ds(r0, _RC)] = (qv[0:D, :] * qscale).astype(bf16)
            vt_scr[:, :, pl.ds(r0, _RC)] = qv[D:2 * D, :].astype(bf16).reshape(H, Dh, _RC)
            return carry

        jax.lax.fori_loop(0, NR, rows, 0)

    q0 = pl.multiple_of(t * TQ, TQ)
    for h in range(H):
        j = h % G
        qm_scr[h, Dh * j:Dh * (j + 1), :] = qt_scr[Dh * h:Dh * (h + 1), pl.ds(q0, TQ)]

    def qk_chunk(u, buf, c, m):
        kc = k_scr[u // G, c * CK:(c + 1) * CK, :]
        s = jnp.dot(kc, qm_scr[u], preferred_element_type=f32)
        buf[c * CK:(c + 1) * CK, :] = s
        return jnp.maximum(m, s.reshape(CK // 8, 8, TQ).max(axis=0))

    def pv_chunk(u, buf, c, mb8, o, l):
        s = buf[c * CK:(c + 1) * CK, :].reshape(CK // 8, 8, TQ)
        p = jnp.exp2(s - mb8[None])
        l = l + p.sum(axis=0)
        vt = vt_scr[u, :, c * CK:(c + 1) * CK]
        o = o + jnp.dot(vt, p.reshape(CK, TQ).astype(bf16), preferred_element_type=f32)
        return o, l

    neg = jnp.full((8, TQ), -jnp.inf, f32)

    def stage(u, cur, nxt, m, do_next=True):
        mb8 = jnp.broadcast_to(m.max(axis=0, keepdims=True), (8, TQ))
        o = jnp.zeros((Dh, TQ), f32)
        l = jnp.zeros((8, TQ), f32)
        mns = [neg]
        for c in range(NC):
            if do_next:
                mns.append(qk_chunk(u + 1, nxt, c, mns[-1]))
            ti = c - _TIE + 1
            if do_next and ti >= 1:
                mbc = mb8 + jnp.minimum(jnp.abs(mns[ti]), 0.0)
            else:
                mbc = mb8
            o, l = pv_chunk(u, cur, c, mbc, o, l)
        r = o / l.sum(axis=0, keepdims=True)
        ot_scr[pl.ds(pl.multiple_of(u * Dh, Dh), Dh), :] = r.astype(ot_scr.dtype)
        return mns[-1]

    m = neg
    for c in range(NC):
        m = qk_chunk(0, sA, c, m)

    bufs = (sA, sB)
    NL = (H - 1) // _U

    def body(i, m):
        for j in range(_U):
            m = stage(_U * i + j, bufs[j % 2], bufs[(j + 1) % 2], m)
        return m

    m = jax.lax.fori_loop(0, NL, body, m)
    for u in range(NL * _U, H):
        m = stage(u, bufs[u % 2], bufs[(u + 1) % 2], m, do_next=(u < H - 1))

    @pl.when(t == 0)
    def _wait_weights():
        for cp in late_copies():
            cp.wait()
        mod_scr[...] = jnp.dot(silu_c(), wmod_ref[:, 2 * D:6 * D],
                               preferred_element_type=f32)[0:8, :]

    ga = mod_scr[0:1, 0:D]
    sb = mod_scr[0:1, D:2 * D]
    cb1 = 1.0 + mod_scr[0:1, 2 * D:3 * D]
    gb = mod_scr[0:1, 3 * D:4 * D]

    o_nat = ot_scr[...].T.astype(bf16)
    attn = jnp.dot(o_nat, wo_ref[...], preferred_element_type=f32)
    x1 = x_ref[pl.ds(q0, TQ), :].astype(f32) + ga * attn
    h2 = (_layernorm(x1) * cb1 + sb).astype(bf16)
    b1 = b1_ref[...].astype(f32).reshape(1, F)
    b2 = b2_ref[...].astype(f32).reshape(1, D)
    acc = jnp.zeros((TQ, D), f32)
    for fc in range(F // _FC):
        u = jnp.dot(h2, w1_ref[:, fc * _FC:(fc + 1) * _FC], preferred_element_type=f32)
        u = u + b1[:, fc * _FC:(fc + 1) * _FC]
        r = jnp.maximum(u, 0.0)
        acc = acc + jnp.dot((r * r).astype(bf16), w2_ref[fc * _FC:(fc + 1) * _FC, :],
                            preferred_element_type=f32)
    out = x1 + gb * (acc + b2)
    o_ref[0] = out.astype(o_ref.dtype)


@jax.jit
def pallas_adaLN_cond__mha_block__dense_activation_squared_relu__prompt_kernel(
    A_x: jax.Array,
    A_wqkv: jax.Array,
    A_wo: jax.Array,
    B_x: jax.Array,
    B_w1: jax.Array,
    B_b1: jax.Array,
    B_w2: jax.Array,
    B_b2: jax.Array,
    c: jax.Array,
    w_mod: jax.Array,
):
    B, S, D = A_x.shape
    F = B_w1.shape[1]
    H = _H
    Dh = D // H

    def full(shape):
        return pl.BlockSpec(shape, lambda t: (0,) * len(shape))

    hbm = pl.BlockSpec(memory_space=pl.ANY)
    return pl.pallas_call(
        functools.partial(_kernel, S=S, D=D, F=F),
        grid=(S // _TQ,),
        in_specs=[hbm, hbm, hbm, hbm, full((F,)), hbm, full((D,)), full((1, D)), hbm],
        out_specs=pl.BlockSpec((1, _TQ, D), lambda t: (0, t, 0)),
        out_shape=jax.ShapeDtypeStruct((B, S, D), A_x.dtype),
        scratch_shapes=[
            pltpu.VMEM((S, D), bf16),
            pltpu.VMEM((D, 3 * D), bf16),
            pltpu.VMEM((D, D), bf16),
            pltpu.VMEM((D, F), bf16),
            pltpu.VMEM((F, D), bf16),
            pltpu.VMEM((D, 6 * D), bf16),
            pltpu.SemaphoreType.DMA((6,)),
            pltpu.SemaphoreType.DMA((S // _RC,)),
            pltpu.VMEM((2 * D, D), bf16),
            pltpu.VMEM((8, 4 * D), f32),
            pltpu.VMEM((D // 128, S, 128), bf16),
            pltpu.VMEM((D, S), bf16),
            pltpu.VMEM((H, Dh, S), bf16),
            pltpu.VMEM((H, 128, _TQ), bf16),
            pltpu.VMEM((S, _TQ), f32),
            pltpu.VMEM((S, _TQ), f32),
            pltpu.VMEM((D, _TQ), f32),
        ],
        compiler_params=pltpu.CompilerParams(
            dimension_semantics=("arbitrary",),
            vmem_limit_bytes=100 * 1024 * 1024,
        ),
    )(A_x, A_wqkv, A_wo, B_w1, B_b1, B_w2, B_b2, c, w_mod)
```

```python
import functools
import math

import jax
import jax.numpy as jnp
import jax.experimental.pallas as pl
import jax.experimental.pallas.tpu as pltpu

f32 = jnp.float32
bf16 = jnp.bfloat16
u32 = jnp.uint32

_H = 32
_EPS = 1e-5
_TQ = 512
_CK = 128
_RC = 1024
_SC = 256
_FC = 256
_TIE = 3
_LAG = 1
_U = 6


def _layernorm(xf):
    mu = jnp.mean(xf, axis=-1, keepdims=True)
    xc = xf - mu
    var = jnp.mean(xc * xc, axis=-1, keepdims=True)
    return xc * jax.lax.rsqrt(var + _EPS)


def _kernel(x_hbm, wqkv_hbm, wo_hbm, w1_hbm, b1_ref, w2_hbm, b2_ref, c_ref, wmod_hbm,
            o_ref,
            x_ref, wqkv_ref, wo_ref, w1_ref, w2_ref, wmod_ref, sems, xsems,
            wqvt_ref, mod_scr, k_scr, qt_scr, vt_scr, qm_scr, sA, sB, ot_scr, m_scr, *, S, D, F):
    t = pl.program_id(0)
    H = _H
    Dh = D // H
    G = 128 // Dh
    NG = D // 128
    TQ, CK = _TQ, _CK
    NC = S // CK
    qscale = (Dh ** -0.5) * math.log2(math.e)

    NR = S // _RC

    def late_copies():
        return [pltpu.make_async_copy(src, dst, sems.at[i]) for i, (src, dst) in enumerate(
            [(wmod_hbm.at[:, 2 * D:6 * D], wmod_ref.at[:, 2 * D:6 * D]),
             (wo_hbm, wo_ref), (w1_hbm, w1_ref), (w2_hbm, w2_ref)])]

    def x_copy(r):
        return pltpu.make_async_copy(x_hbm.at[0, pl.ds(r * _RC, _RC), :],
                                     x_ref.at[pl.ds(r * _RC, _RC), :], xsems.at[r])

    def silu_c():
        cf = c_ref[...].astype(f32)
        return jnp.broadcast_to(cf * jax.nn.sigmoid(cf), (16, D)).astype(bf16)

    @pl.when(t == 0)
    def _prologue():
        cp_mod = pltpu.make_async_copy(wmod_hbm.at[:, 0:2 * D], wmod_ref.at[:, 0:2 * D], sems.at[4])
        cp_qkv = pltpu.make_async_copy(wqkv_hbm, wqkv_ref, sems.at[5])
        cp_qkv.start()
        cp_mod.start()
        for r in range(NR):
            x_copy(r).start()
        qm_scr[...] = jnp.zeros(qm_scr.shape, qm_scr.dtype)
        cp_qkv.wait()
        wqvt_ref[0:D, :] = wqkv_ref[:, 0:D].T
        wqvt_ref[D:2 * D, :] = wqkv_ref[:, 2 * D:3 * D].T
        cp_mod.wait()
        mod = jnp.dot(silu_c(), wmod_ref[:, 0:2 * D], preferred_element_type=f32)
        for cp in late_copies():
            cp.start()

        sa = mod[0:1, 0:D]
        ca1 = 1.0 + mod[0:1, D:2 * D]

        def rows(r, carry):
            x_copy(r).wait()
            for sub in range(_RC // _SC):
                r0 = pl.multiple_of(r * _RC + sub * _SC, _SC)
                r0h = pl.multiple_of(r * (_RC // 2) + sub * (_SC // 2), _SC // 2)
                xf = x_ref[pl.ds(r0, _SC), :].astype(f32)
                h = (_layernorm(xf) * ca1 + sa).astype(bf16)
                k = jnp.dot(h, wqkv_ref[:, D:2 * D], preferred_element_type=f32).astype(bf16)
                for g in range(NG):
                    k_scr[g, pl.ds(r0h, _SC // 2), :] = pltpu.bitcast(k[:, 128 * g:128 * (g + 1)], u32)
                qv = jax.lax.dot_general(wqvt_ref[...], h, (((1,), (1,)), ((), ())),
                                         preferred_element_type=f32)
                qt_scr[:, pl.ds(r0, _SC)] = (qv[0:D, :] * qscale).astype(bf16)
                vt_scr[:, :, pl.ds(r0, _SC)] = pltpu.bitcast(
                    qv[D:2 * D, :].astype(bf16), u32).reshape(H, Dh // 2, _SC)
            return carry

        jax.lax.fori_loop(0, NR, rows, 0)

    q0 = pl.multiple_of(t * TQ, TQ)
    neg = jnp.full((8, TQ), -jnp.inf, f32)

    def set_qm(slot, h, qstart):
        j = h % G
        qm_scr[slot, Dh // 2 * j:Dh // 2 * (j + 1), :] = pltpu.bitcast(
            qt_scr[Dh * h:Dh * (h + 1), pl.ds(qstart, TQ)], u32)

    def qk_chunk(slot, buf, c, m):
        kc = pltpu.bitcast(k_scr[(slot // G) % NG, c * CK // 2:(c + 1) * CK // 2, :], bf16)
        s = jnp.dot(kc, pltpu.bitcast(qm_scr[slot], bf16),
                    preferred_element_type=f32)
        buf[c * CK:(c + 1) * CK, :] = s
        return jnp.maximum(m, s.reshape(CK // 8, 8, TQ).max(axis=0))

    @pl.when(t == 0)
    def _first_scores():
        set_qm(0, 0, 0)
        m = neg
        for c in range(NC):
            m = qk_chunk(0, sA, c, m)
        m_scr[...] = m

    for h in range(1, H):
        set_qm(h, h, q0)
    set_qm(H, 0, pl.multiple_of(jnp.minimum(t + 1, pl.num_programs(0) - 1) * TQ, TQ))

    def pv_chunk(u, buf, c, mb8, o, l):
        s = buf[c * CK:(c + 1) * CK, :].reshape(CK // 8, 8, TQ)
        p = jnp.exp2(s - mb8[None])
        l = l + p.sum(axis=0)
        vt = pltpu.bitcast(vt_scr[u, :, c * CK:(c + 1) * CK], bf16)
        o = o + jnp.dot(vt, p.reshape(CK, TQ).astype(bf16), preferred_element_type=f32)
        return o, l

    bufs = (sA, sB)

    def run(u0, n, m):
        ms = {0: m}
        prog = []
        st = {}

        def pv(p):
            j, c = divmod(p, NC)
            if c == 0:
                st[j] = (jnp.broadcast_to(ms[j].max(axis=0, keepdims=True), (8, TQ)),
                         jnp.zeros((Dh, TQ), f32), jnp.zeros((8, TQ), f32))
            mb8, o, l = st[j]
            ti = min(p + _LAG - _TIE, len(prog) - 1)
            mbc = mb8 + jnp.minimum(jnp.abs(prog[ti]), 0.0) if ti >= 0 else mb8
            o, l = pv_chunk(u0 + j, bufs[j % 2], c, mbc, o, l)
            st[j] = (mb8, o, l)
            if c == NC - 1:
                r = o / l.sum(axis=0, keepdims=True)
                ot_scr[pl.ds(pl.multiple_of((u0 + j) * Dh, Dh), Dh), :] = r.astype(ot_scr.dtype)

        for j in range(n):
            mn = neg
            for c in range(NC):
                mn = qk_chunk(u0 + j + 1, bufs[(j + 1) % 2], c, mn)
                prog.append(mn)
                if j * NC + c - _LAG >= 0:
                    pv(j * NC + c - _LAG)
            ms[j + 1] = mn
        for p in range(n * NC - _LAG, n * NC):
            pv(p)
        return ms[n]

    NL = (H - 1) // _U
    m = jax.lax.fori_loop(0, NL, lambda i, m: run(_U * i, _U, m), m_scr[...])

    @pl.when(t == 0)
    def _wait_weights():
        for cp in late_copies():
            cp.wait()
        mod_scr[...] = jnp.dot(silu_c(), wmod_ref[:, 2 * D:6 * D],
                               preferred_element_type=f32)[0:8, :]

    m_scr[...] = run(NL * _U, H - NL * _U, m)

    ga = mod_scr[0:1, 0:D]
    sb = mod_scr[0:1, D:2 * D]
    cb1 = 1.0 + mod_scr[0:1, 2 * D:3 * D]
    gb = mod_scr[0:1, 3 * D:4 * D]

    o_nat = ot_scr[...].T.astype(bf16)
    attn = jnp.dot(o_nat, wo_ref[...], preferred_element_type=f32)
    x1 = x_ref[pl.ds(q0, TQ), :].astype(f32) + ga * attn
    h2 = (_layernorm(x1) * cb1 + sb).astype(bf16)
    b1 = b1_ref[...].astype(f32).reshape(1, F)
    b2 = b2_ref[...].astype(f32).reshape(1, D)
    acc = jnp.zeros((TQ, D), f32)
    for fc in range(F // _FC):
        u = jnp.dot(h2, w1_ref[:, fc * _FC:(fc + 1) * _FC], preferred_element_type=f32)
        u = u + b1[:, fc * _FC:(fc + 1) * _FC]
        r = jnp.maximum(u, 0.0)
        acc = acc + jnp.dot((r * r).astype(bf16), w2_ref[fc * _FC:(fc + 1) * _FC, :],
                            preferred_element_type=f32)
    out = x1 + gb * (acc + b2)
    o_ref[0] = out.astype(o_ref.dtype)


@jax.jit
def pallas_adaLN_cond__mha_block__dense_activation_squared_relu__prompt_kernel(
    A_x: jax.Array,
    A_wqkv: jax.Array,
    A_wo: jax.Array,
    B_x: jax.Array,
    B_w1: jax.Array,
    B_b1: jax.Array,
    B_w2: jax.Array,
    B_b2: jax.Array,
    c: jax.Array,
    w_mod: jax.Array,
):
    B, S, D = A_x.shape
    F = B_w1.shape[1]
    H = _H
    Dh = D // H

    def full(shape):
        return pl.BlockSpec(shape, lambda t: (0,) * len(shape))

    hbm = pl.BlockSpec(memory_space=pl.ANY)
    return pl.pallas_call(
        functools.partial(_kernel, S=S, D=D, F=F),
        grid=(S // _TQ,),
        in_specs=[hbm, hbm, hbm, hbm, full((F,)), hbm, full((D,)), full((1, D)), hbm],
        out_specs=pl.BlockSpec((1, _TQ, D), lambda t: (0, t, 0)),
        out_shape=jax.ShapeDtypeStruct((B, S, D), A_x.dtype),
        scratch_shapes=[
            pltpu.VMEM((S, D), bf16),
            pltpu.VMEM((D, 3 * D), bf16),
            pltpu.VMEM((D, D), bf16),
            pltpu.VMEM((D, F), bf16),
            pltpu.VMEM((F, D), bf16),
            pltpu.VMEM((D, 6 * D), bf16),
            pltpu.SemaphoreType.DMA((6,)),
            pltpu.SemaphoreType.DMA((S // _RC,)),
            pltpu.VMEM((2 * D, D), bf16),
            pltpu.VMEM((8, 4 * D), f32),
            pltpu.VMEM((D // 128, S // 2, 128), u32),
            pltpu.VMEM((D, S), bf16),
            pltpu.VMEM((H, Dh // 2, S), u32),
            pltpu.VMEM((H + 1, 64, _TQ), u32),
            pltpu.VMEM((S, _TQ), f32),
            pltpu.VMEM((S, _TQ), f32),
            pltpu.VMEM((D, _TQ), f32),
            pltpu.VMEM((8, _TQ), f32),
        ],
        compiler_params=pltpu.CompilerParams(
            dimension_semantics=("arbitrary",),
            vmem_limit_bytes=100 * 1024 * 1024,
        ),
    )(A_x, A_wqkv, A_wo, B_w1, B_b1, B_w2, B_b2, c, w_mod)
```
